```python
import jax
import jax.numpy as jnp

def _softmax(x, axis=-1):
    return jax.nn.softmax(x, axis=axis)
def _gelu(x):
    return jax.nn.gelu(x, approximate=True)
def _silu(x):
    return jax.nn.silu(x)
def _sigmoid(x):
    return jax.nn.sigmoid(x)
def _layernorm(x, axis=-1, eps=1e-5):
    m = jnp.mean(x, axis=axis, keepdims=True)
    v = jnp.var(x, axis=axis, keepdims=True)
    return (x - m) / jnp.sqrt(v + eps)
def _scatter_add(tgt, idx, src, axis=0):
    return tgt.at[idx].add(src)
def _segment_sum(src, seg, n):
    return jax.ops.segment_sum(src, seg, n)
class _Rng:
    def __init__(self, key):
        self._k = key
    def _next(self):
        self._k, sub = jax.random.split(self._k)
        return sub
    def normal(self, shape):
        return jax.random.normal(self._next(), shape, dtype=jnp.bfloat16)
    def randint(self, lo, hi, shape):
        return jax.random.randint(self._next(), shape, lo, hi, dtype=jnp.int32)
    def uniform(self, shape, lo=0.0, hi=1.0):
        return jax.random.uniform(self._next(), shape, jnp.bfloat16, lo, hi)
    def permutation(self, n):
        return jax.random.permutation(self._next(), n)


kernel_name = 'parallel_sum__sliding_block_cached__glu_gated_swiglu__decode'

def setup_inputs():
    _rng = _Rng(jax.random.key(int.from_bytes(__import__("os").urandom(4), "little")))
    _w = (lambda a: (lambda t: t.astype(jnp.bfloat16) if jnp.issubdtype(t.dtype, jnp.floating) else t)(jnp.asarray(a)))
    def _A_setup():
        B, Sq, D = 4, 1, 640
        Hq, Hkv, Sk, Dh = 32, 32, 8192, 192
        assert Hq % Hkv == 0, (Hq, Hkv)
        return {
            "x": _w((lambda *s: _rng.normal(s) * 0.05)(B, Sq, D)),
            "k_cache": _w((lambda *s: _rng.normal(s) * 0.05)(B, Hkv, Sk, Dh)),
            "v_cache": _w((lambda *s: _rng.normal(s) * 0.05)(B, Hkv, Sk, Dh)),
            "wq": _w((lambda *s: _rng.normal(s) * 0.05)(D, Hq * Dh) * (D ** -0.5)),
            "wo": _w((lambda *s: _rng.normal(s) * 0.05)(Hq * Dh, D) * ((Hq * Dh) ** -0.5)),
        }
    _A_in = _A_setup()

    def _B_setup():
        B, S, D, F = 4, 1, 640, 1536
        return {
            "x": _w((lambda *s: _rng.normal(s) * 0.05)(B, S, D)),
            "w1": _w((lambda *s: _rng.normal(s) * 0.05)(D, F) * (2.0 / D) ** 0.5),
            "w3": _w((lambda *s: _rng.normal(s) * 0.05)(D, F) * (2.0 / D) ** 0.5),
            "w2": _w((lambda *s: _rng.normal(s) * 0.05)(F, D) * (2.0 / F) ** 0.5),
        }
    _B_in = _B_setup()

    return {
        "A_x": _A_in["x"],
        "A_k_cache": _A_in["k_cache"],
        "A_v_cache": _A_in["v_cache"],
        "A_wq": _A_in["wq"],
        "A_wo": _A_in["wo"],
        "B_x": _B_in["x"],
        "B_w1": _B_in["w1"],
        "B_w3": _B_in["w3"],
        "B_w2": _B_in["w2"],
    }

def reference(A_x, A_k_cache, A_v_cache, A_wq, A_wo, B_x, B_w1, B_w3, B_w2):
    def _A_ref(x, k_cache, v_cache, wq, wo):
        B, Sq, D = x.shape
        Hq, Dh = 32, 192
        Hkv, Sk = k_cache.shape[1], k_cache.shape[2]
        W = min(4096, max(256, Sk // 4))
        rep = Hq // Hkv
        q = (lambda x, *d: x.transpose(*d))((x @ wq).reshape(B, Sq, Hq, Dh), 0, 2, 1, 3)
        k = jnp.repeat(k_cache[:, :, Sk - W:, :], rep, axis=1)
        v = jnp.repeat(v_cache[:, :, Sk - W:, :], rep, axis=1)
        scores = jnp.einsum("bhqd,bhkd->bhqk", q, k) * (Dh ** -0.5)
        p = _softmax(scores, axis=-1)
        o = jnp.einsum("bhqk,bhkd->bhqd", p, v)
        return (lambda x, *d: x.transpose(*d))(o, 0, 2, 1, 3).reshape(B, Sq, Hq * Dh) @ wo

    def _B_ref(x, w1, w3, w2):
        gate = jnp.einsum("bsd,df->bsf", x, w1)
        up = jnp.einsum("bsd,df->bsf", x, w3)
        h = _silu(gate) * up
        out = jnp.einsum("bsf,fd->bsd", h, w2)
        return out

    x = A_x
    xn = _layernorm(x, axis=-1)
    return x + _A_ref(xn, A_k_cache, A_v_cache, A_wq, A_wo) + _B_ref(xn, B_w1, B_w3, B_w2)
```

```python
import jax
import jax.numpy as jnp
from jax import lax
import jax.experimental.pallas as pl
import jax.experimental.pallas.tpu as pltpu

B, H, SK, DH, D, F, W = 4, 32, 8192, 192, 640, 1536, 2048
NP = H // 2
NH = 2
ffn_at = 1
f32, bf16 = jnp.float32, jnp.bfloat16

class _Two:
    def __init__(self, c): self.c = c
    def start(self, priority):
        self.c[0].start(priority=priority); self.c[1].start(priority=1 - priority)
    def wait(self):
        self.c[0].wait(); self.c[1].wait()


def kern(x_hbm, k_hbm, v_hbm, wq_hbm, wo_hbm, w1_hbm, w3_hbm, w2_hbm, o_ref,
         kbuf, vbuf, wqbuf, wobuf, w1buf, w3buf, w2buf, acc_ref, x_ref, xsem, ksem, vsem, wqsem, wosem, fsem):
  def kcp(h, b):
      s = h % NH
      return _Two([pltpu.make_async_copy(k_hbm.at[b, h, pl.ds(r, 96), pl.ds(SK - W, W)], kbuf.at[s, b, pl.ds(r, 96)], ksem.at[s, b]) for r in (0, 96)])
  def vcp(h, b):
      s = h % NH
      return _Two([pltpu.make_async_copy(v_hbm.at[b, h, pl.ds(r, 96), pl.ds(SK - W, W)], vbuf.at[s, b, pl.ds(r, 96)], vsem.at[s, b]) for r in (0, 96)])
  def wqcp(j):
      return pltpu.make_async_copy(wq_hbm.at[:, pl.ds(pl.multiple_of(j * 2 * DH, 128), 2 * DH)], wqbuf.at[j % 2], wqsem.at[j % 2])
  def wocp(j):
      return pltpu.make_async_copy(wo_hbm.at[pl.ds(pl.multiple_of(j * 2 * DH, 128), 2 * DH), :], wobuf.at[j % 2], wosem.at[j % 2])
  fcp = [pltpu.make_async_copy(s, d, fsem.at[i]) for i, (s, d) in
         enumerate([(w1_hbm, w1buf), (w3_hbm, w3buf), (w2_hbm, w2buf)])]

  xc_ = pltpu.make_async_copy(x_hbm, x_ref, xsem); xc_.start()
  wqcp(0).start()
  for h in range(NH):
      for b in range(B): kcp(h, b).start(priority=0)
      for b in range(B): vcp(h, b).start(priority=0)
      if h == 0:
          wocp(0).start()
          for c in fcp: c.start()

  xc_.wait()
  x = x_ref[...].astype(f32)
  m = jnp.mean(x, axis=-1, keepdims=True)
  xc = x - m
  var = jnp.mean(xc * xc, axis=-1, keepdims=True)
  xn = (xc / jnp.sqrt(var + 1e-5)).astype(bf16)
  acc_ref[...] = x
  row_s = lax.broadcasted_iota(jnp.int32, (B, W), 0)
  row_o = lax.broadcasted_iota(jnp.int32, (B, DH), 0)

  def pair(j, _):
      @pl.when(j + 1 < NP)
      def _(): wqcp(j + 1).start()
      wqcp(j).wait()
      qp = jnp.dot(xn, wqbuf[j % 2], preferred_element_type=f32).astype(bf16)
      upd = None
      for t in range(2):
          h = 2 * j + t
          sl = h % NH
          q = qp[:, t * DH:(t + 1) * DH]
          s = None
          for b in range(B):
              kcp(h, b).wait()
              sb = jnp.dot(q, kbuf[sl, b], preferred_element_type=f32)
              s = sb if b == 0 else jnp.where(row_s == b, sb, s)
              @pl.when(h + NH < H)
              def _(): kcp(h + NH, b).start(priority=0)
          s = s * (DH ** -0.5)
          e = jnp.exp(s - jnp.max(s, axis=-1, keepdims=True))
          l = jnp.sum(e, axis=-1, keepdims=True)
          p = e.astype(bf16)
          o = None
          for b in range(B):
              vcp(h, b).wait()
              ob = lax.dot_general(p, vbuf[sl, b], (((1,), (1,)), ((), ())), preferred_element_type=f32)
              o = ob if b == 0 else jnp.where(row_o == b, ob, o)
              @pl.when(h + NH < H)
              def _(): vcp(h + NH, b).start(priority=0)
          o = (o / l).astype(bf16)
          if t == 0: wocp(j).wait()
          u = jnp.dot(o, wobuf[j % 2, t * DH:(t + 1) * DH, :], preferred_element_type=f32)
          upd = u if t == 0 else upd + u
      acc_ref[...] += upd
      @pl.when(j + 2 < NP)
      def _(): wocp(j + 2).start()
      @pl.when(j == 0)
      def _(): wocp(1).start()
      @pl.when(j == ffn_at)
      def _():
          for c in fcp: c.wait()
          g = jnp.dot(xn, w1buf[...], preferred_element_type=f32)
          up = jnp.dot(xn, w3buf[...], preferred_element_type=f32)
          hh = (g * jax.nn.sigmoid(g) * up).astype(bf16)
          acc_ref[...] += jnp.dot(hh, w2buf[...], preferred_element_type=f32)
  lax.fori_loop(0, NP, pair, None)
  o_ref[...] = acc_ref[...].astype(o_ref.dtype)

@jax.jit
def pallas_parallel_sum__sliding_block_cached__glu_gated_swiglu__decode_kernel(A_x, A_k_cache, A_v_cache, A_wq, A_wo, B_x, B_w1, B_w3, B_w2):
  any_spec = pl.BlockSpec(memory_space=pl.ANY)
  out = pl.pallas_call(
      kern,
      out_shape=jax.ShapeDtypeStruct((B, D), bf16),
      in_specs=[any_spec] * 8,
      out_specs=pl.BlockSpec(memory_space=pltpu.VMEM),
      scratch_shapes=[
          pltpu.VMEM((NH, B, DH, W), bf16), pltpu.VMEM((NH, B, DH, W), bf16),
          pltpu.VMEM((2, D, 2 * DH), bf16), pltpu.VMEM((2, 2 * DH, D), bf16),
          pltpu.VMEM((D, F), bf16), pltpu.VMEM((D, F), bf16), pltpu.VMEM((F, D), bf16),
          pltpu.VMEM((B, D), f32), pltpu.VMEM((B, D), bf16), pltpu.SemaphoreType.DMA(()),
          pltpu.SemaphoreType.DMA((NH, B)), pltpu.SemaphoreType.DMA((NH, B)),
          pltpu.SemaphoreType.DMA((2,)), pltpu.SemaphoreType.DMA((2,)), pltpu.SemaphoreType.DMA((3,)),
      ],
      compiler_params=pltpu.CompilerParams(vmem_limit_bytes=100 << 20),
  )(A_x.reshape(B, D), jnp.swapaxes(A_k_cache, 2, 3), jnp.swapaxes(A_v_cache, 2, 3),
    A_wq, A_wo, B_w1, B_w3, B_w2)
  return out.reshape(B, 1, D)
```
